```python
import os as _os
_os.environ.setdefault("JAX_PLATFORMS", "cpu")
import jax
import jax.numpy as jnp

def _softmax(x, axis=-1):
    return jax.nn.softmax(x, axis=axis)
def _gelu(x):
    return jax.nn.gelu(x, approximate=True)
def _silu(x):
    return jax.nn.silu(x)
def _sigmoid(x):
    return jax.nn.sigmoid(x)
def _layernorm(x, axis=-1, eps=1e-5):
    m = jnp.mean(x, axis=axis, keepdims=True)
    v = jnp.var(x, axis=axis, keepdims=True)
    return (x - m) / jnp.sqrt(v + eps)
def _scatter_add(tgt, idx, src, axis=0):
    return tgt.at[idx].add(src)
def _segment_sum(src, seg, n):
    return jax.ops.segment_sum(src, seg, n)
class _Rng:
    def __init__(self, key):
        self._k = key
    def _next(self):
        self._k, sub = jax.random.split(self._k)
        return sub
    def normal(self, shape):
        return jax.random.normal(self._next(), shape, dtype=jnp.bfloat16)
    def randint(self, lo, hi, shape):
        return jax.random.randint(self._next(), shape, lo, hi, dtype=jnp.int32)
    def uniform(self, shape, lo=0.0, hi=1.0):
        return jax.random.uniform(self._next(), shape, jnp.bfloat16, lo, hi)
    def permutation(self, n):
        return jax.random.permutation(self._next(), n)


kernel_name = 'concat_heads__mha_block__ssm_conv_s4__prompt'

def setup_inputs():
    _rng = _Rng(jax.random.key(int.from_bytes(__import__("os").urandom(4), "little")))
    _w = (lambda a: (lambda t: t.astype(jnp.bfloat16) if jnp.issubdtype(t.dtype, jnp.floating) else t)(jnp.asarray(a)))
    def _A_setup():
        B, S, D, H = 1, 2048, 448, 16
        return {
            "x": _w((lambda *s: _rng.normal(s) * 0.2)(B, S, D)),
            "wqkv": _w((lambda *s: _rng.normal(s) * 0.2)(D, 3 * D)),
            "wo": _w((lambda *s: _rng.normal(s) * 0.05)(D, D)),
        }
    _A_in = _A_setup()

    def _B_setup():
        B, L, D, N = 1, 2048, 448, 256
        A_re = -jnp.exp((lambda *s: _rng.normal(s) * 0.2)(D, N))
        A_im = jnp.pi * (lambda *s: _rng.normal(s) * 0.2)(D, N)
        B_re = (lambda *s: _rng.normal(s) * 0.2)(D, N)
        B_im = (lambda *s: _rng.normal(s) * 0.2)(D, N)
        C_re = (lambda *s: _rng.normal(s) * 0.2)(D, N)
        C_im = (lambda *s: _rng.normal(s) * 0.2)(D, N)
        log_dt = (lambda *s: _rng.normal(s) * 0.2)(D) * 0.5 - 4.0
        Dskip = (lambda *s: _rng.normal(s) * 0.05)(D)
        return {
            "u": _w((lambda *s: _rng.normal(s) * 0.05)(B, L, D)),
            "A_re": _w(A_re),
            "A_im": _w(A_im),
            "B_re": _w(B_re),
            "B_im": _w(B_im),
            "C_re": _w(C_re),
            "C_im": _w(C_im),
            "log_dt": _w(log_dt),
            "Dskip": _w(Dskip),
        }
    _B_in = _B_setup()

    return {
        "A_x": _A_in["x"],
        "A_wqkv": _A_in["wqkv"],
        "A_wo": _A_in["wo"],
        "B_u": _B_in["u"],
        "B_A_re": _B_in["A_re"],
        "B_A_im": _B_in["A_im"],
        "B_B_re": _B_in["B_re"],
        "B_B_im": _B_in["B_im"],
        "B_C_re": _B_in["C_re"],
        "B_C_im": _B_in["C_im"],
        "B_log_dt": _B_in["log_dt"],
        "B_Dskip": _B_in["Dskip"],
    }

def reference(A_x, A_wqkv, A_wo, B_u, B_A_re, B_A_im, B_B_re, B_B_im, B_C_re, B_C_im, B_log_dt, B_Dskip):
    def _A_ref(x, wqkv, wo):
        B, S, D = x.shape
        H = 16
        Dh = D // H
        qkv = (lambda x, *d: x.transpose(*d))((x @ wqkv).reshape(B, S, 3, H, Dh), 2, 0, 3, 1, 4)
        q, k, v = qkv[0], qkv[1], qkv[2]
        scores = jnp.einsum("bhqd,bhkd->bhqk", q, k) * (Dh ** -0.5)
        p = _softmax(scores, axis=-1)
        o = jnp.einsum("bhqk,bhkd->bhqd", p, v)
        return (lambda x, *d: x.transpose(*d))(o, 0, 2, 1, 3).reshape(B, S, D) @ wo

    def _B_ref(u, A_re, A_im, B_re, B_im, C_re, C_im, log_dt, Dskip):
        Bsz, L, D = u.shape
        dt = jnp.exp(log_dt)[:, None]
        A = A_re + 1j * A_im
        Bc = B_re + 1j * B_im
        Cc = C_re + 1j * C_im
        logdA = dt * A
        dB = dt * Bc
        l = (lambda x, dt: x.astype(dt))(jnp.arange(L), A_re.dtype)
        P = jnp.exp(logdA[:, :, None] * l[None, None, :])
        K = jnp.einsum("dn,dnl,dn->dl", Cc, P, dB).real
        L2 = 2 * L
        Kp = jnp.pad(K, ((0, 0), (0, L)))
        up = (lambda x, *d: x.transpose(*d))(u, 0, 2, 1)
        up = jnp.pad(up, ((0, 0), (0, 0), (0, L)))
        Kf = (lambda x, axes=(-2,-1): jnp.fft.rfft2(x.astype(jnp.float32), axes=axes))(Kp[:, None, :], axes=(-2, -1))
        Uf = (lambda x, axes=(-2,-1): jnp.fft.rfft2(x.astype(jnp.float32), axes=axes))(up[:, :, None, :], axes=(-2, -1))
        Yf = Uf * Kf[None, :, :, :]
        y = (lambda x, s, axes=(-2,-1): jnp.fft.irfft2(x, s=s, axes=axes).astype(jnp.bfloat16))(Yf, (1, L2), axes=(-2, -1))[:, :, 0, :L]
        y = (lambda x, *d: x.transpose(*d))(y, 0, 2, 1) + u * Dskip[None, None, :]
        return y

    a = _A_ref(A_x, A_wqkv, A_wo)
    b = _B_ref(B_u, B_A_re, B_A_im, B_B_re, B_B_im, B_C_re, B_C_im, B_log_dt, B_Dskip)
    return jnp.concatenate([a, b], axis=-1)
```

```python
import functools

import jax
import jax.numpy as jnp
import numpy as np
import jax.experimental.pallas as pl
import jax.experimental.pallas.tpu as pltpu

F32 = jnp.float32
BF16 = jnp.bfloat16

S = 2048
D = 448
H = 16
DH = 28
DHP = 32
NG = 4
N = 256
CB = 128
NB = S // CB
KD_ROWS = 768
TQ = 256


def _bf16_round(x):
    x = np.ascontiguousarray(x, dtype=np.float32)
    u = x.view(np.uint32)
    r = (u + 0x7FFF + ((u >> 16) & 1)) & 0xFFFF0000
    return r.astype(np.uint32).view(np.float32)


def _split_hi_lo(m):
    hi = _bf16_round(m)
    lo = _bf16_round(m.astype(np.float64) - hi.astype(np.float64))
    return hi, lo


@functools.lru_cache(maxsize=1)
def _constants():
    th = np.pi * (2 * np.arange(CB) + 1) / (2 * CB)
    t = np.arange(2 * CB)
    ffwd = np.concatenate([np.cos(th[:, None] * t[None, :CB]),
                           -np.sin(th[:, None] * t[None, :CB])], 0)
    finv = np.concatenate([np.cos(th[None, :] * t[CB:, None]),
                           -np.sin(th[None, :] * t[CB:, None])], 1) / CB
    r = _bf16_round(np.arange(S, dtype=np.float32)).astype(np.int64)
    pts = np.concatenate([np.arange(256), 256 + 2 * np.arange(128), 512 + 4 * np.arange(128),
                          1024 + 8 * np.arange(128), [2048]]).astype(np.int64)
    row = np.searchsorted(pts, r)
    assert np.all(pts[row] == r)
    g = np.zeros((NB, 2 * CB, 2 * CB), np.float64)
    base, nk = [], []
    for c in range(NB):
        ls = np.arange(CB * (c - 1), CB * (c + 1))
        ls = ls[ls >= 0]
        rows = row[ls]
        b = (rows.min() // CB) * CB
        k = (rows.max() - b) // CB + 1
        assert k <= 2
        base.append(int(b)); nk.append(int(k))
        tt = ls - CB * (c - 1)
        for l_t, rr in zip(tt, rows):
            g[c, :CB, rr - b] += np.cos(th * l_t)
            g[c, CB:, rr - b] += -np.sin(th * l_t)
    fh, fl = _split_hi_lo(ffwd)
    ih, il = _split_hi_lo(finv)
    gh, gl = _split_hi_lo(g)
    return (fh, fl, ih, il, gh, gl, tuple(base), tuple(nk))


def _kernel(x_ref, wqkv_ref, wo_ref, u_ref, ar_ref, ai_ref, br_ref, bi_ref, cr_ref, ci_ref,
            ldt_ref, dsk_ref, fh_ref, fl_ref, ih_ref, il_ref, gh_ref, gl_ref,
            out_ref,
            qkv_scr, vm_scr, o_scr, kd_scr, uh_scr, kh_scr, z_scr, *, gbase, gnk):

    def qkv_body(i, c):
        r0 = pl.multiple_of(i * TQ, TQ)
        acc = jnp.dot(x_ref[pl.ds(r0, TQ), :], wqkv_ref[...], preferred_element_type=F32)
        lane = jax.lax.broadcasted_iota(jnp.int32, acc.shape, 1)
        acc = jnp.where(lane < H * DHP, acc * (DH ** -0.5), acc)
        qkv_scr[pl.ds(r0, TQ), :] = acc.astype(BF16)
        return c

    jax.lax.fori_loop(0, S // TQ, qkv_body, 0)

    lane128 = jax.lax.broadcasted_iota(jnp.int32, (1, 128), 1)

    for g in range(NG):
        vg = qkv_scr[:, pl.ds(2 * H * DHP + g * 128, 128)]
        for hh in range(4):
            m = (lane128 // DHP) == hh
            vm_scr[hh] = jnp.where(m, vg, jnp.zeros_like(vg))

        def attn_body(i, c, g=g):
            r0 = pl.multiple_of(i * TQ, TQ)
            qg = qkv_scr[pl.ds(r0, TQ), pl.ds(g * 128, 128)]
            kg = qkv_scr[:, pl.ds(H * DHP + g * 128, 128)]
            og = jnp.zeros((TQ, 128), F32)
            for hh in range(4):
                m = (lane128 // DHP) == hh
                qm = jnp.where(m, qg, jnp.zeros_like(qg))
                s = jax.lax.dot_general(qm, kg, (((1,), (1,)), ((), ())),
                                        preferred_element_type=F32)
                mx = jnp.max(s, axis=-1, keepdims=True)
                p = jnp.exp(s - mx)
                l = jnp.sum(p, axis=-1, keepdims=True)
                pv = jnp.dot(p.astype(BF16), vm_scr[hh], preferred_element_type=F32)
                og = og + pv * (1.0 / l)
            o_scr[pl.ds(r0, TQ), pl.ds(g * 128, 128)] = og.astype(BF16)
            return c

        jax.lax.fori_loop(0, S // TQ, attn_body, 0)

    dt = jnp.exp(ldt_ref[...].astype(F32)).astype(BF16).astype(F32)
    z_scr[0] = dt * ar_ref[...].astype(F32)
    z_scr[1] = dt * ai_ref[...].astype(F32)
    dbr = dt * br_ref[...].astype(F32)
    dbi = dt * bi_ref[...].astype(F32)
    cr = cr_ref[...].astype(F32)
    ci = ci_ref[...].astype(F32)
    z_scr[2] = cr * dbr - ci * dbi
    z_scr[3] = cr * dbi + ci * dbr
    kd_scr[...] = jnp.zeros(kd_scr.shape, F32)

    srow = jax.lax.broadcasted_iota(jnp.int32, (8, D), 0)
    sf = srow.astype(F32)
    mexp = jnp.zeros((8, D), F32)
    for j, mv in enumerate((8, 16, 32, 64, 256, 512, 1024, 2048)):
        mexp = jnp.where(srow == j, float(mv), mexp)

    def kgen_body(n, c):
        zr = z_scr[0, pl.ds(n, 1), :]
        zi = z_scr[1, pl.ds(n, 1), :]
        wr = z_scr[2, pl.ds(n, 1), :]
        wi = z_scr[3, pl.ds(n, 1), :]
        er = jnp.exp(zr * sf)
        e_re = er * jnp.cos(zi * sf)
        e_im = er * jnp.sin(zi * sf)
        rr = jnp.exp(zr * mexp)
        r_re = rr * jnp.cos(zi * mexp)
        r_im = rr * jnp.sin(zi * mexp)
        row = 0
        for seg in range(4):
            if seg == 0:
                sr, si = wr, wi
            else:
                pr, pi_ = r_re[3 + seg:4 + seg], r_im[3 + seg:4 + seg]
                sr, si = wr * pr - wi * pi_, wr * pi_ + wi * pr
                e_re, e_im = e_re * e_re - e_im * e_im, 2.0 * e_re * e_im
            x0r = sr * e_re - si * e_im
            x0i = sr * e_im + si * e_re
            qr, qi = r_re[seg:seg + 1], r_im[seg:seg + 1]
            x1r = x0r * qr - x0i * qi
            a = 2.0 * qr
            b = rr[seg:seg + 1] * rr[seg:seg + 1]
            nblk = 32 if seg == 0 else (16 if seg < 3 else 17)
            xp, xc = x0r, x1r
            kd_scr[pl.ds(row, 8), :] += xp
            row += 8
            for k in range(1, nblk):
                kd_scr[pl.ds(row, 8), :] += xc
                row += 8
                if k + 1 < nblk:
                    xp, xc = xc, a * xc - b * xp
        return c

    jax.lax.fori_loop(0, N, kgen_body, 0)
    tail = kd_scr[pl.ds(640, 8), :]
    kd_scr[pl.ds(640, 8), :] = jnp.where(srow == 0, tail, 0.0)

    fh = fh_ref[...]
    fl = fl_ref[...]

    def udft_body(i, c):
        r0 = pl.multiple_of(i * CB, CB)
        ub = u_ref[pl.ds(r0, CB), :]
        uh_scr[i] = (jnp.dot(fh, ub, preferred_element_type=F32)
                     + jnp.dot(fl, ub, preferred_element_type=F32))
        return c

    jax.lax.fori_loop(0, NB, udft_body, 0)

    for c in range(NB):
        kk = gnk[c] * CB
        kd = kd_scr[pl.ds(gbase[c], kk), :]
        kd_hi = kd.astype(BF16)
        kd_lo = (kd - kd_hi.astype(F32)).astype(BF16)
        gh = gh_ref[c, :, pl.ds(0, kk)]
        gl = gl_ref[c, :, pl.ds(0, kk)]
        kh_scr[c] = (jnp.dot(gh, kd_hi, preferred_element_type=F32)
                     + jnp.dot(gh, kd_lo, preferred_element_type=F32)
                     + jnp.dot(gl, kd_hi, preferred_element_type=F32))

    ih = ih_ref[...]
    il = il_ref[...]
    dsk = dsk_ref[...].astype(F32)
    wo = wo_ref[...]

    def conv_body(i, c):
        def inner(cc, acc):
            yr, yi = acc
            kr = kh_scr[cc, pl.ds(0, CB), :]
            ki = kh_scr[cc, pl.ds(CB, CB), :]
            ur = uh_scr[i - cc, pl.ds(0, CB), :]
            ui = uh_scr[i - cc, pl.ds(CB, CB), :]
            return yr + (kr * ur - ki * ui), yi + (kr * ui + ki * ur)

        z0 = jnp.zeros((CB, D), F32)
        yr, yi = jax.lax.fori_loop(0, i + 1, inner, (z0, z0))
        yh = jnp.concatenate([yr, yi], axis=0)
        yh_hi = yh.astype(BF16)
        yh_lo = (yh - yh_hi.astype(F32)).astype(BF16)
        y = (jnp.dot(ih, yh_hi, preferred_element_type=F32)
             + jnp.dot(ih, yh_lo, preferred_element_type=F32)
             + jnp.dot(il, yh_hi, preferred_element_type=F32))
        r0 = pl.multiple_of(i * CB, CB)
        ub = u_ref[pl.ds(r0, CB), :].astype(F32)
        t1 = (ub * dsk).astype(BF16).astype(F32)
        ob = (y.astype(BF16).astype(F32) + t1).astype(BF16)
        oa = jnp.dot(o_scr[pl.ds(r0, CB), :], wo, preferred_element_type=F32).astype(BF16)
        out_ref[pl.ds(r0, CB), :] = jnp.concatenate([oa, ob], axis=1)
        return c

    jax.lax.fori_loop(0, NB, conv_body, 0)


@jax.jit
def pallas_concat_heads__mha_block__ssm_conv_s4__prompt_kernel(
    A_x, A_wqkv, A_wo, B_u, B_A_re, B_A_im, B_B_re, B_B_im, B_C_re, B_C_im, B_log_dt, B_Dskip,
):
    fh, fl, ih, il, gh, gl, gbase, gnk = _constants()
    x = A_x.reshape(S, D)
    u = B_u.reshape(S, D)
    wqkv = jnp.pad(A_wqkv.reshape(D, 3, H, DH), ((0, 0), (0, 0), (0, 0), (0, DHP - DH)))
    wqkv = wqkv.reshape(D, 3 * H * DHP)
    wo = jnp.pad(A_wo.reshape(H, DH, D), ((0, 0), (0, DHP - DH), (0, 0))).reshape(H * DHP, D)
    tr = lambda a: a.T
    consts = [jnp.asarray(c, dtype=BF16) for c in (fh, fl, ih, il, gh, gl)]
    out = pl.pallas_call(
        functools.partial(_kernel, gbase=gbase, gnk=gnk),
        out_shape=jax.ShapeDtypeStruct((S, 2 * D), BF16),
        scratch_shapes=[
            pltpu.VMEM((S, 3 * H * DHP), BF16),
            pltpu.VMEM((4, S, 128), BF16),
            pltpu.VMEM((S, H * DHP), BF16),
            pltpu.VMEM((KD_ROWS, D), F32),
            pltpu.VMEM((NB, 2 * CB, D), F32),
            pltpu.VMEM((NB, 2 * CB, D), F32),
            pltpu.VMEM((4, N, D), F32),
        ],
        compiler_params=pltpu.CompilerParams(vmem_limit_bytes=100 * 1024 * 1024),
    )(x, wqkv, wo, u, tr(B_A_re), tr(B_A_im), tr(B_B_re), tr(B_B_im), tr(B_C_re), tr(B_C_im),
      B_log_dt.reshape(1, D), B_Dskip.reshape(1, D), *consts)
    return out.reshape(1, S, 2 * D)
```

```python
import functools

import jax
import jax.numpy as jnp
import numpy as np
import jax.experimental.pallas as pl
import jax.experimental.pallas.tpu as pltpu

F32 = jnp.float32
BF16 = jnp.bfloat16

S = 2048
D = 448
H = 16
DH = 28
DHP = 32
NG = 4
N = 256
CB = 128
NB = S // CB
KD_ROWS = 768
TQ = 512
NQB = S // TQ
NSTEP = NQB * H
NPS = N // NSTEP
LOG2E = 1.4426950408889634
DP = 512


def _bf16_round(x):
    x = np.ascontiguousarray(x, dtype=np.float32)
    u = x.view(np.uint32)
    r = (u + 0x7FFF + ((u >> 16) & 1)) & 0xFFFF0000
    return r.astype(np.uint32).view(np.float32)


def _split_hi_lo(m):
    hi = _bf16_round(m)
    lo = _bf16_round(m.astype(np.float64) - hi.astype(np.float64))
    return hi, lo


@functools.lru_cache(maxsize=1)
def _constants():
    th = np.pi * (2 * np.arange(CB) + 1) / (2 * CB)
    t = np.arange(2 * CB)
    ffwd = np.concatenate([np.cos(th[:, None] * t[None, :CB]),
                           -np.sin(th[:, None] * t[None, :CB])], 0)
    finv = np.concatenate([np.cos(th[None, :] * t[CB:, None]),
                           -np.sin(th[None, :] * t[CB:, None])], 1) / CB
    r = _bf16_round(np.arange(S, dtype=np.float32)).astype(np.int64)
    pts = np.concatenate([np.arange(256), 256 + 2 * np.arange(128), 512 + 4 * np.arange(128),
                          1024 + 8 * np.arange(128), [2048]]).astype(np.int64)
    row = np.searchsorted(pts, r)
    assert np.all(pts[row] == r)
    g = np.zeros((NB, 2 * CB, 2 * CB), np.float64)
    base, nk = [], []
    for c in range(NB):
        ls = np.arange(CB * (c - 1), CB * (c + 1))
        ls = ls[ls >= 0]
        rows = row[ls]
        b = (rows.min() // CB) * CB
        k = (rows.max() - b) // CB + 1
        assert k <= 2
        base.append(int(b)); nk.append(int(k))
        tt = ls - CB * (c - 1)
        for l_t, rr in zip(tt, rows):
            g[c, :CB, rr - b] += np.cos(th * l_t)
            g[c, CB:, rr - b] += -np.sin(th * l_t)
    fh, fl = _split_hi_lo(ffwd)
    ih, il = _split_hi_lo(finv)
    gh, gl = _split_hi_lo(g)
    f2 = np.concatenate([fh, fl], 1)
    i3 = np.concatenate([ih, ih, il], 1)
    return (f2, i3, gh, gl, tuple(base), tuple(nk))


def _kernel(x_ref, wqk_ref, wvt_ref, wo_ref, u_ref, ar_ref, ai_ref, br_ref, bi_ref, cr_ref, ci_ref,
            ldt_ref, dsk_ref, f2_ref, i3_ref, gh_ref, gl_ref,
            out_ref,
            q_scr, k_scr, vt_scr, st_scr, ot_scr, oa_scr, kd_scr, uh_scr, kh_scr, yh_scr, z_scr, *, gbase, gnk):
    def qkv_body(i, c):
        r0 = pl.multiple_of(i * TQ, TQ)
        xb = x_ref[pl.ds(r0, TQ), :]
        acc = jnp.dot(xb, wqk_ref[...], preferred_element_type=F32)
        for g in range(NG):
            q_scr[g, pl.ds(r0, TQ), :] = (acc[:, g * 128:(g + 1) * 128]
                                          * (DH ** -0.5 * LOG2E)).astype(BF16)
            k_scr[g, pl.ds(r0, TQ), :] = acc[:, 512 + g * 128:512 + (g + 1) * 128].astype(BF16)
        vt = jax.lax.dot_general(wvt_ref[...], xb, (((1,), (1,)), ((), ())),
                                 preferred_element_type=F32)
        rowi = jax.lax.broadcasted_iota(jnp.int32, vt.shape, 0)
        vt = jnp.where((rowi % DHP) == DH, 1.0, vt).astype(BF16)
        for h in range(H):
            vt_scr[h, :, pl.ds(r0, TQ)] = vt[h * DHP:(h + 1) * DHP, :]
        return c

    with jax.named_scope('qkv'):
        jax.lax.fori_loop(0, NQB, qkv_body, 0)

    dt = jnp.exp(ldt_ref[...].astype(F32)).astype(BF16).astype(F32)
    srow = jax.lax.broadcasted_iota(jnp.int32, (8, D), 0)
    lane128 = jax.lax.broadcasted_iota(jnp.int32, (1, 128), 1)

    def prep_body(i, c):
        r0 = pl.multiple_of(i * 8, 8)
        rows = pl.ds(r0, 8)
        zr = dt * ar_ref[rows, :].astype(F32)
        zi = dt * ai_ref[rows, :].astype(F32)
        dbr = dt * br_ref[rows, :].astype(F32)
        dbi = dt * bi_ref[rows, :].astype(F32)
        cr = cr_ref[rows, :].astype(F32)
        ci = ci_ref[rows, :].astype(F32)
        z_scr[20, rows, pl.ds(0, D)] = cr * dbr - ci * dbi
        z_scr[21, rows, pl.ds(0, D)] = cr * dbi + ci * dbr

        def ev(m):
            e = jnp.exp(zr * m)
            return e * jnp.cos(zi * m), e * jnp.sin(zi * m)

        def sq(p):
            return p[0] * p[0] - p[1] * p[1], 2.0 * p[0] * p[1]

        p1 = ev(1.0); p2 = sq(p1); p4 = sq(p2)
        p8 = ev(8.0); p16 = sq(p8); p32 = sq(p16); p64 = sq(p32)
        p256 = ev(256.0); p512 = sq(p256); p1024 = sq(p512)
        for j, p in enumerate((p1, p2, p4, p8, p16, p32, p64, p256, p512, p1024)):
            z_scr[2 * j, rows, pl.ds(0, D)] = p[0]
            z_scr[2 * j + 1, rows, pl.ds(0, D)] = p[1]
        return c

    with jax.named_scope('prep'):
        z_scr[:, :, pl.ds(384, 128)] = jnp.zeros((22, N, 128), F32)
        jax.lax.fori_loop(0, N // 8, prep_body, 0)
        kd_scr[...] = jnp.zeros(kd_scr.shape, F32)

    srow128 = jax.lax.broadcasted_iota(jnp.int32, (8, 128), 0)

    def kgen_setup(n, col, pin):
        lanes = pl.ds(col * 128, 128)

        def row(j):
            return pin(jnp.broadcast_to(z_scr[j, pl.ds(n, 1), :][:, col * 128:(col + 1) * 128], (8, 128)))

        def cmul(a, b):
            return a[0] * b[0] - a[1] * b[1], a[0] * b[1] + a[1] * b[0]

        def pick(bit, j):
            m = (srow128 & bit) != 0
            return jnp.where(m, row(2 * j), 1.0), jnp.where(m, row(2 * j + 1), 0.0)

        e = cmul(cmul(pick(1, 0), pick(2, 1)), pick(4, 2))
        w = (row(20), row(21))
        segs = []
        for seg in range(4):
            if seg == 0:
                st = w
            else:
                st = cmul(w, (row(2 * (6 + seg)), row(2 * (6 + seg) + 1)))
                e = (e[0] * e[0] - e[1] * e[1], 2.0 * e[0] * e[1])
            x0 = cmul(st, e)
            qr, qi = row(2 * (3 + seg)), row(2 * (3 + seg) + 1)
            x1r = x0[0] * qr - x0[1] * qi
            segs.append((x0[0], x1r, 2.0 * qr, qr * qr + qi * qi))
        return segs

    def kgen_pieces(n0, npiece):
        work = []
        tokens = [None]

        def pin(x):
            if tokens[0] is None:
                return x
            t = tokens[0]
            return jnp.where(t > jnp.inf, t, x)
        for col in range(DP // 128):
            lanes = pl.ds(col * 128, 128)
            state = {}

            def setup(col=col, state=state):
                state['st'] = [kgen_setup(n0 + j, col, pin) for j in range(NPS)]
                tokens[0] = None

            work.append(setup)
            row = 0
            for seg in range(4):
                nblk = 32 if seg == 0 else (16 if seg < 3 else 17)
                for k in range(nblk):
                    def blk(seg=seg, k=k, nblk=nblk, row=row, lanes=lanes, state=state):
                        st = state['st']
                        if k == 0:
                            state['xs'] = [(s_[seg][0], s_[seg][1]) for s_ in st]
                        xs = [(pin(xp), pin(xc)) for xp, xc in state['xs']]
                        tokens[0] = None
                        tot = xs[0][0]
                        for j in range(1, NPS):
                            tot = tot + xs[j][0]
                        kd_scr[pl.ds(row, 8), lanes] += tot
                        if k + 1 < nblk:
                            state['xs'] = [(xc, st[j][seg][2] * xc - st[j][seg][3] * xp)
                                           if k + 2 < nblk else (xc, xc)
                                           for j, (xp, xc) in enumerate(xs)]
                    work.append(blk)
                    row += 8
        per = -(-len(work) // npiece)
        for p in range(npiece):
            tok = yield
            tokens[0] = tok
            for w in work[p * per:(p + 1) * per]:
                w()
        yield

    NCH = 1
    TPC = 128
    KC = S // NCH

    def q_masked(step):
        qb = step // H
        h = step % H
        r0 = pl.multiple_of(qb * TQ, TQ)
        qg = q_scr[h // 4, pl.ds(r0, TQ), :]
        return jnp.where((lane128 // DHP) == (h % 4), qg, jnp.zeros_like(qg))

    def scores_chunk(step, qm, ch):
        g = (step % H) // 4
        st = jax.lax.dot_general(k_scr[g, pl.ds(ch * KC, KC), :], qm, (((1,), (1,)), ((), ())),
                                 preferred_element_type=F32)
        st_scr[step % 2, pl.ds(ch * KC, KC), :] = st
        return jnp.max(st, axis=0, keepdims=True)

    def step_body(step, mx):
        qb = step // H
        h = step % H
        r0 = pl.multiple_of(qb * TQ, TQ)
        nstep = jnp.minimum(step + 1, NSTEP - 1)
        qm = q_masked(nstep)
        pieces = kgen_pieces(step * NPS, NCH * TPC)
        next(pieces)
        mx_next = None
        ot = None
        for ch in range(NCH):
            m = scores_chunk(nstep, qm, ch)
            mx_next = m if mx_next is None else jnp.maximum(mx_next, m)
            st = st_scr[step % 2, pl.ds(ch * KC, KC), :]
            pt = jnp.exp2(st - mx).astype(BF16)
            o = jnp.dot(vt_scr[h, :, pl.ds(ch * KC, KC)], pt, preferred_element_type=F32)
            ot = o if ot is None else ot + o
            for tk in range(TPC):
                pieces.send(st_scr[nstep % 2, pl.ds(ch * KC + tk * (KC // TPC), 8), pl.ds(0, 128)])
        ot = ot * (1.0 / ot[DH:DH + 1, :])
        ot_scr[pl.ds(pl.multiple_of(h * DHP, DHP), DHP), :] = ot.astype(BF16)

        @pl.when(h == H - 1)
        def _():
            oa = jax.lax.dot_general(ot_scr[...], wo_ref[...], (((0,), (0,)), ((), ())),
                                     preferred_element_type=F32)
            oa_scr[pl.ds(r0, TQ), :] = oa.astype(BF16)
        return mx_next

    with jax.named_scope('attn_kgen'):
        qm0 = q_masked(0)
        mx0 = scores_chunk(0, qm0, 0)
        for ch in range(1, NCH):
            mx0 = jnp.maximum(mx0, scores_chunk(0, qm0, ch))
        jax.lax.fori_loop(0, NSTEP, step_body, mx0)

    tail = kd_scr[pl.ds(640, 8), pl.ds(0, D)]
    kd_scr[pl.ds(640, 8), pl.ds(0, D)] = jnp.where(srow == 0, tail, 0.0)

    def udft_body(i, c):
        r0 = pl.multiple_of(i * CB, CB)
        ub = u_ref[pl.ds(r0, CB), :]
        uh_scr[i] = jnp.dot(f2_ref[...], jnp.concatenate([ub, ub], axis=0),
                            preferred_element_type=F32)
        return c

    with jax.named_scope('udft'):
        jax.lax.fori_loop(0, NB, udft_body, 0)

    with jax.named_scope('kdft'):
        for c in range(NB):
            kk = gnk[c] * CB
            kd = kd_scr[pl.ds(gbase[c], kk), pl.ds(0, D)]
            kd_hi = kd.astype(BF16)
            kd_lo = (kd - kd_hi.astype(F32)).astype(BF16)
            gh = gh_ref[c, :, pl.ds(0, kk)]
            gl = gl_ref[c, :, pl.ds(0, kk)]
            kh_scr[c] = jnp.dot(jnp.concatenate([gh, gh, gl], axis=1),
                                jnp.concatenate([kd_hi, kd_lo, kd_hi], axis=0),
                                preferred_element_type=F32)

    dsk = dsk_ref[...].astype(F32)

    def acc_body(rb, c):
        rows_r = pl.ds(pl.multiple_of(rb * 8, 8), 8)
        rows_i = pl.ds(pl.multiple_of(CB + rb * 8, 8), 8)
        for i in range(NB):
            yr = yi = None
            for cc in range(i + 1):
                kr = kh_scr[cc, rows_r, :]
                ki = kh_scr[cc, rows_i, :]
                ur = uh_scr[i - cc, rows_r, :]
                ui = uh_scr[i - cc, rows_i, :]
                tr_ = kr * ur - ki * ui
                ti_ = kr * ui + ki * ur
                yr = tr_ if yr is None else yr + tr_
                yi = ti_ if yi is None else yi + ti_
            yh_scr[i, rows_r, :] = yr
            yh_scr[i, rows_i, :] = yi
        return c

    with jax.named_scope('cacc'):
        jax.lax.fori_loop(0, CB // 8, acc_body, 0)

    def conv_body(i, c):
        yh = yh_scr[i]
        yh_hi = yh.astype(BF16)
        yh_lo = (yh - yh_hi.astype(F32)).astype(BF16)
        y = jnp.dot(i3_ref[...], jnp.concatenate([yh_hi, yh_lo, yh_hi], axis=0),
                    preferred_element_type=F32)
        r0 = pl.multiple_of(i * CB, CB)
        ub = u_ref[pl.ds(r0, CB), :].astype(F32)
        t1 = (ub * dsk).astype(BF16).astype(F32)
        ob = (y.astype(BF16).astype(F32) + t1).astype(BF16)
        out_ref[pl.ds(r0, CB), :] = jnp.concatenate([oa_scr[pl.ds(r0, CB), :], ob], axis=1)
        return c

    with jax.named_scope('conv'):
        jax.lax.fori_loop(0, NB, conv_body, 0)


@jax.jit
def pallas_concat_heads__mha_block__ssm_conv_s4__prompt_kernel(
    A_x, A_wqkv, A_wo, B_u, B_A_re, B_A_im, B_B_re, B_B_im, B_C_re, B_C_im, B_log_dt, B_Dskip,
):
    f2, i3, gh, gl, gbase, gnk = _constants()
    x = A_x.reshape(S, D)
    u = B_u.reshape(S, D)
    wp = jnp.pad(A_wqkv.reshape(D, 3, H, DH), ((0, 0), (0, 0), (0, 0), (0, DHP - DH)))
    wqk = wp[:, :2].reshape(D, 2 * H * DHP)
    wvt = wp[:, 2].reshape(D, H * DHP).T
    wo = jnp.pad(A_wo.reshape(H, DH, D), ((0, 0), (0, DHP - DH), (0, 0))).reshape(H * DHP, D)
    tr = lambda a: a.T
    consts = [jnp.asarray(c, dtype=BF16) for c in (f2, i3, gh, gl)]
    out = pl.pallas_call(
        functools.partial(_kernel, gbase=gbase, gnk=gnk),
        out_shape=jax.ShapeDtypeStruct((S, 2 * D), BF16),
        scratch_shapes=[
            pltpu.VMEM((NG, S, 128), BF16),
            pltpu.VMEM((NG, S, 128), BF16),
            pltpu.VMEM((H, DHP, S), BF16),
            pltpu.VMEM((2, S, TQ), F32),
            pltpu.VMEM((H * DHP, TQ), BF16),
            pltpu.VMEM((S, D), BF16),
            pltpu.VMEM((KD_ROWS, DP), F32),
            pltpu.VMEM((NB, 2 * CB, D), F32),
            pltpu.VMEM((NB, 2 * CB, D), F32),
            pltpu.VMEM((NB, 2 * CB, D), F32),
            pltpu.VMEM((22, N, DP), F32),
        ],
        compiler_params=pltpu.CompilerParams(vmem_limit_bytes=100 * 1024 * 1024),
    )(x, wqk, wvt, wo, u, tr(B_A_re), tr(B_A_im), tr(B_B_re), tr(B_B_im), tr(B_C_re), tr(B_C_im),
      B_log_dt.reshape(1, D), B_Dskip.reshape(1, D), *consts)
    return out.reshape(1, S, 2 * D)
```

```python
import functools

import jax
import jax.numpy as jnp
import numpy as np
import jax.experimental.pallas as pl
import jax.experimental.pallas.tpu as pltpu

F32 = jnp.float32
BF16 = jnp.bfloat16

S = 2048
D = 448
H = 16
DH = 28
DHP = 32
NG = 4
N = 256
CB = 128
NB = S // CB
KD_ROWS = 656
TQ = 512
NQB = S // TQ
NSTEP = NQB * H
NPS = N // NSTEP
TPC = 128
LOG2E = 1.4426950408889634
DP = 512


def _bf16_round(x):
    x = np.ascontiguousarray(x, dtype=np.float32)
    u = x.view(np.uint32)
    r = (u + 0x7FFF + ((u >> 16) & 1)) & 0xFFFF0000
    return r.astype(np.uint32).view(np.float32)


def _split_hi_lo(m):
    hi = _bf16_round(m)
    lo = _bf16_round(m.astype(np.float64) - hi.astype(np.float64))
    return hi, lo


@functools.lru_cache(maxsize=1)
def _constants():
    th = np.pi * (2 * np.arange(CB) + 1) / (2 * CB)
    t = np.arange(2 * CB)
    ffwd = np.concatenate([np.cos(th[:, None] * t[None, :CB]),
                           -np.sin(th[:, None] * t[None, :CB])], 0)
    finv = np.concatenate([np.cos(th[None, :] * t[CB:, None]),
                           -np.sin(th[None, :] * t[CB:, None])], 1) / CB
    r = _bf16_round(np.arange(S, dtype=np.float32)).astype(np.int64)
    pts = np.concatenate([np.arange(256), 256 + 2 * np.arange(128), 512 + 4 * np.arange(128),
                          1024 + 8 * np.arange(128), [2048]]).astype(np.int64)
    row = np.searchsorted(pts, r)
    assert np.all(pts[row] == r)
    blocks, meta, off = [], [], 0
    for c in range(NB):
        ls = np.arange(CB * (c - 1), CB * (c + 1))
        ls = ls[ls >= 0]
        rows = row[ls]
        b = int(rows.min() // 16) * 16
        n = -(-(int(rows.max()) + 1 - b) // 16) * 16
        g = np.zeros((2 * CB, n), np.float64)
        tt = ls - CB * (c - 1)
        for l_t, rr in zip(tt, rows):
            g[:CB, rr - b] += np.cos(th * l_t)
            g[CB:, rr - b] += -np.sin(th * l_t)
        gh, gl = _split_hi_lo(g)
        w = -(-2 * n // 128) * 128
        blk = np.zeros((2 * CB, w), np.float32)
        blk[:, :n] = gh
        blk[:, n:2 * n] = gl
        blocks.append(blk)
        meta.append((b, n, off))
        off += w
    fh, fl = _split_hi_lo(ffwd)
    ih, il = _split_hi_lo(finv)
    f2 = np.concatenate([fh, fl], 1)
    i3 = np.concatenate([ih, ih, il], 1)
    return (f2, i3, np.concatenate(blocks, 1), tuple(meta))


def _kernel(x_hbm, wt_hbm, wo_hbm, u_hbm, ar_ref, ai_ref, br_ref, bi_ref, cr_ref, ci_ref,
            ldt_ref, dsk_ref, f2_ref, i3_ref, g_hbm,
            out_hbm,
            x_ref, wt_ref, wo_ref, ut_ref, u_ref, g_ref, obuf, in_sems, out_sems,
            q_scr, k_scr, vt_scr, st_scr, ot_scr, oa_scr, kd_scr, uh_scr, kh_scr, yh_scr,
            p_scr, z_scr, *, gmeta):
    copies = [pltpu.make_async_copy(src, dst, in_sems.at[i]) for i, (src, dst) in enumerate(
        ((x_hbm, x_ref), (wt_hbm, wt_ref), (wo_hbm, wo_ref), (u_hbm, ut_ref), (g_hbm, g_ref)))]
    for cp in copies:
        cp.start()

    def pin(tok, x):
        return jnp.where(tok > jnp.inf, tok, x)

    for j, r in enumerate((ar_ref, ai_ref, br_ref, bi_ref, cr_ref, ci_ref)):
        p_scr[j] = r[...].astype(F32).T
    dt = jnp.exp(ldt_ref[...].astype(F32)).astype(BF16).astype(F32)
    srow = jax.lax.broadcasted_iota(jnp.int32, (8, D), 0)
    row128 = jax.lax.broadcasted_iota(jnp.int32, (128, 1), 0)
    z_scr[:, :, pl.ds(384, 128)] = jnp.zeros((22, N, 128), F32)
    kd_scr[...] = jnp.zeros(kd_scr.shape, F32)

    def prep_block(i, tok):
        rows = pl.ds(pl.multiple_of(i * 8, 8), 8)
        dtp = jnp.concatenate([pin(tok, jnp.broadcast_to(dt[:, :128], (8, 128))),
                               jnp.broadcast_to(dt[:, 128:], (8, D - 128))], axis=1)
        zr = dtp * p_scr[0, rows, :]
        zi = dtp * p_scr[1, rows, :]
        dbr = dtp * p_scr[2, rows, :]
        dbi = dtp * p_scr[3, rows, :]
        cr = p_scr[4, rows, :]
        ci = p_scr[5, rows, :]
        z_scr[20, rows, pl.ds(0, D)] = cr * dbr - ci * dbi
        z_scr[21, rows, pl.ds(0, D)] = cr * dbi + ci * dbr

        def ev(m):
            e = jnp.exp(zr * m)
            return e * jnp.cos(zi * m), e * jnp.sin(zi * m)

        def sq(p):
            return p[0] * p[0] - p[1] * p[1], 2.0 * p[0] * p[1]

        p1 = ev(1.0); p2 = sq(p1); p4 = sq(p2)
        p8 = sq(p4); p16 = sq(p8); p32 = sq(p16); p64 = sq(p32)
        p256 = ev(256.0); p512 = sq(p256); p1024 = sq(p512)
        for j, p in enumerate((p1, p2, p4, p8, p16, p32, p64, p256, p512, p1024)):
            z_scr[2 * j, rows, pl.ds(0, D)] = p[0]
            z_scr[2 * j + 1, rows, pl.ds(0, D)] = p[1]

    copies[0].wait(); copies[1].wait(); copies[3].wait()
    u_ref[:, pl.ds(384, 128)] = jnp.zeros((S, 128), BF16)
    PPB = N // 8 // NQB

    def qkv_body(i, c):
        r0 = pl.multiple_of(i * TQ, TQ)
        acc = jnp.dot(wt_ref[...], x_ref[:, pl.ds(r0, TQ)], preferred_element_type=F32)
        for g in range(NG):
            q_scr[g, :, pl.ds(r0, TQ)] = (acc[g * 128:(g + 1) * 128, :]
                                          * (DH ** -0.5 * LOG2E)).astype(BF16)
            k_scr[g, pl.ds(r0, TQ), :] = acc[512 + g * 128:512 + (g + 1) * 128, :].T.astype(BF16)
        vt = acc[1024:, :]
        rowi = jax.lax.broadcasted_iota(jnp.int32, vt.shape, 0)
        vtb = jnp.where((rowi % DHP) == DH, 1.0, vt).astype(BF16)
        for h in range(H):
            vt_scr[h, :, pl.ds(r0, TQ)] = vtb[h * DHP:(h + 1) * DHP, :]
        for j in range(TQ // CB):
            c0 = pl.multiple_of(r0 + j * CB, CB)
            u_ref[pl.ds(c0, CB), pl.ds(0, D)] = ut_ref[:, pl.ds(c0, CB)].astype(F32).T.astype(BF16)
        for j in range(PPB):
            rr = j * (1536 // PPB)
            prep_block(i * PPB + j, acc[rr:rr + 8, 0:128])
        return c

    with jax.named_scope('qkv'):
        jax.lax.fori_loop(0, NQB, qkv_body, 0)

    srow128 = jax.lax.broadcasted_iota(jnp.int32, (8, 128), 0)

    def kgen_setup(n, col, pn):
        def row(j):
            return pn(jnp.broadcast_to(z_scr[j, pl.ds(n, 1), :][:, col * 128:(col + 1) * 128],
                                       (8, 128)))

        def cmul(a, b):
            return a[0] * b[0] - a[1] * b[1], a[0] * b[1] + a[1] * b[0]

        def pick(bit, j):
            m = (srow128 & bit) != 0
            return jnp.where(m, row(2 * j), 1.0), jnp.where(m, row(2 * j + 1), 0.0)

        e = cmul(cmul(pick(1, 0), pick(2, 1)), pick(4, 2))
        w = (row(20), row(21))
        segs = []
        for seg in range(4):
            if seg == 0:
                st = w
            else:
                st = cmul(w, (row(2 * (6 + seg)), row(2 * (6 + seg) + 1)))
                e = (e[0] * e[0] - e[1] * e[1], 2.0 * e[0] * e[1])
            x0 = cmul(st, e)
            qr, qi = row(2 * (3 + seg)), row(2 * (3 + seg) + 1)
            x1r = x0[0] * qr - x0[1] * qi
            segs.append((x0[0], x1r, 2.0 * qr, qr * qr + qi * qi))
        return segs

    def kgen_pieces(n0, npiece):
        work = []
        tokens = [None]

        def pn(x):
            return x if tokens[0] is None else pin(tokens[0], x)

        for col in range(DP // 128):
            lanes = pl.ds(col * 128, 128)
            state = {}

            def setup(col=col, state=state):
                state['st'] = [kgen_setup(n0 + j, col, pn) for j in range(NPS)]
                tokens[0] = None

            work.append(setup)
            row = 0
            for seg in range(4):
                nblk = 32 if seg == 0 else (16 if seg < 3 else 17)
                for k in range(nblk):
                    def blk(seg=seg, k=k, nblk=nblk, row=row, lanes=lanes, state=state):
                        st = state['st']
                        if k == 0:
                            state['xs'] = [(s_[seg][0], s_[seg][1]) for s_ in st]
                        xs = [(xp, pn(xc)) for xp, xc in state['xs']]
                        tokens[0] = None
                        tot = xs[0][0]
                        for j in range(1, NPS):
                            tot = tot + xs[j][0]
                        kd_scr[pl.ds(row, 8), lanes] += tot
                        if k + 1 < nblk:
                            state['xs'] = [(xc, st[j][seg][2] * xc - st[j][seg][3] * xp)
                                           if k + 2 < nblk else (xc, xc)
                                           for j, (xp, xc) in enumerate(xs)]
                    work.append(blk)
                    row += 8
        per = -(-len(work) // npiece)
        for p in range(npiece):
            tok = yield
            tokens[0] = tok
            for w in work[p * per:(p + 1) * per]:
                w()
        yield

    def scores(step):
        qb = step // H
        h = step % H
        r0 = pl.multiple_of(qb * TQ, TQ)
        qg = q_scr[h // 4, :, pl.ds(r0, TQ)]
        qm = jnp.where((row128 // DHP) == (h % 4), qg, jnp.zeros_like(qg))
        st = jnp.dot(k_scr[h // 4], qm, preferred_element_type=F32)
        st_scr[step % 2] = st
        return jnp.max(st, axis=0, keepdims=True)

    def step_body(step, mx):
        qb = step // H
        h = step % H
        r0 = pl.multiple_of(qb * TQ, TQ)
        nstep = jnp.minimum(step + 1, NSTEP - 1)
        pieces = kgen_pieces(step * NPS, TPC)
        next(pieces)
        pt = jnp.exp2(st_scr[step % 2] - mx).astype(BF16)
        ot = jnp.dot(vt_scr[h], pt, preferred_element_type=F32)
        mx_next = scores(nstep)
        ulanes = pl.ds(pl.multiple_of((step % 4) * 128, 128), 128)
        ub = u_ref[pl.ds(pl.multiple_of((step // 4) * CB, CB), CB), ulanes]
        uh_scr[step // 4, :, ulanes] = jnp.dot(f2_ref[...], jnp.concatenate([ub, ub], axis=0),
                                               preferred_element_type=F32)
        for tk in range(TPC):
            pieces.send(st_scr[nstep % 2, pl.ds(tk * (S // TPC), 8), pl.ds(0, 128)])
        ot = ot * (1.0 / ot[DH:DH + 1, :])
        ot_scr[pl.ds(pl.multiple_of(h * DHP, DHP), DHP), :] = ot.astype(BF16)

        @pl.when(h == H - 1)
        def _():
            oa = jax.lax.dot_general(ot_scr[...], wo_ref[...], (((0,), (0,)), ((), ())),
                                     preferred_element_type=F32)
            oa_scr[pl.ds(r0, TQ), :] = oa.astype(BF16)
        return mx_next

    copies[2].wait()
    with jax.named_scope('attn_kgen'):
        jax.lax.fori_loop(0, NSTEP, step_body, scores(0))

    tail = kd_scr[pl.ds(640, 8), pl.ds(0, D)]
    kd_scr[pl.ds(640, 8), pl.ds(0, D)] = jnp.where(srow == 0, tail, 0.0)

    copies[4].wait()

    with jax.named_scope('kdft'):
        for c in range(NB):
            b, n, off = gmeta[c]
            kd = kd_scr[pl.ds(b, n), pl.ds(0, D)]
            kd_hi = kd.astype(BF16)
            kd_lo = (kd - kd_hi.astype(F32)).astype(BF16)
            g2 = g_ref[:, pl.ds(off, 2 * n)]
            kh_scr[c] = (jnp.dot(g2, jnp.concatenate([kd_hi, kd_hi], axis=0),
                                 preferred_element_type=F32)
                         + jnp.dot(g2[:, :n], kd_lo, preferred_element_type=F32))

    dsk = dsk_ref[...].astype(F32)

    def acc_body(rb, c):
        rows_r = pl.ds(pl.multiple_of(rb * 8, 8), 8)
        rows_i = pl.ds(pl.multiple_of(CB + rb * 8, 8), 8)
        for i in range(NB):
            yr = yi = None
            for cc in range(i + 1):
                kr = kh_scr[cc, rows_r, :]
                ki = kh_scr[cc, rows_i, :]
                ur = uh_scr[i - cc, rows_r, pl.ds(0, D)]
                ui = uh_scr[i - cc, rows_i, pl.ds(0, D)]
                tr_ = kr * ur - ki * ui
                ti_ = kr * ui + ki * ur
                yr = tr_ if yr is None else yr + tr_
                yi = ti_ if yi is None else yi + ti_
            yh_scr[i, rows_r, :] = yr
            yh_scr[i, rows_i, :] = yi
        return c

    with jax.named_scope('cacc'):
        jax.lax.fori_loop(0, CB // 8, acc_body, 0)

    def out_copy(i, slot):
        return pltpu.make_async_copy(obuf.at[slot],
                                     out_hbm.at[pl.ds(pl.multiple_of(i * CB, CB), CB), :],
                                     out_sems.at[slot])

    def conv_body(i, c):
        slot = i % 2
        yh = yh_scr[i]
        yh_hi = yh.astype(BF16)
        yh_lo = (yh - yh_hi.astype(F32)).astype(BF16)
        y = jnp.dot(i3_ref[...], jnp.concatenate([yh_hi, yh_lo, yh_hi], axis=0),
                    preferred_element_type=F32)
        r0 = pl.multiple_of(i * CB, CB)
        ub = u_ref[pl.ds(r0, CB), pl.ds(0, D)].astype(F32)
        t1 = (ub * dsk).astype(BF16).astype(F32)
        ob = (y.astype(BF16).astype(F32) + t1).astype(BF16)

        @pl.when(i >= 2)
        def _():
            out_copy(i - 2, slot).wait()

        obuf[slot] = jnp.concatenate([oa_scr[pl.ds(r0, CB), :], ob], axis=1)
        out_copy(i, slot).start()
        return c

    with jax.named_scope('conv'):
        jax.lax.fori_loop(0, NB, conv_body, 0)
    out_copy(NB - 2, 0).wait()
    out_copy(NB - 1, 1).wait()


@jax.jit
def pallas_concat_heads__mha_block__ssm_conv_s4__prompt_kernel(
    A_x, A_wqkv, A_wo, B_u, B_A_re, B_A_im, B_B_re, B_B_im, B_C_re, B_C_im, B_log_dt, B_Dskip,
):
    f2, i3, gt, gmeta = _constants()
    xt = A_x.reshape(S, D).T
    ut = B_u.reshape(S, D).T
    wt = jnp.pad(A_wqkv.T.reshape(3 * H, DH, D), ((0, 0), (0, DHP - DH), (0, 0))).reshape(3 * H * DHP, D)
    wo = jnp.pad(A_wo.reshape(H, DH, D), ((0, 0), (0, DHP - DH), (0, 0))).reshape(H * DHP, D)
    consts = [jnp.asarray(c, dtype=BF16) for c in (f2, i3, gt)]
    hbm = pl.BlockSpec(memory_space=pl.ANY)
    vmem = pl.BlockSpec(memory_space=pltpu.VMEM)
    out = pl.pallas_call(
        functools.partial(_kernel, gmeta=gmeta),
        out_shape=jax.ShapeDtypeStruct((S, 2 * D), BF16),
        in_specs=[hbm] * 4 + [vmem] * 10 + [hbm],
        out_specs=hbm,
        scratch_shapes=[
            pltpu.VMEM((D, S), BF16),
            pltpu.VMEM((3 * H * DHP, D), BF16),
            pltpu.VMEM((H * DHP, D), BF16),
            pltpu.VMEM((D, S), BF16),
            pltpu.VMEM((S, DP), BF16),
            pltpu.VMEM(gt.shape, BF16),
            pltpu.VMEM((2, CB, 2 * D), BF16),
            pltpu.SemaphoreType.DMA((5,)),
            pltpu.SemaphoreType.DMA((2,)),
            pltpu.VMEM((NG, 128, S), BF16),
            pltpu.VMEM((NG, S, 128), BF16),
            pltpu.VMEM((H, DHP, S), BF16),
            pltpu.VMEM((2, S, TQ), F32),
            pltpu.VMEM((H * DHP, TQ), BF16),
            pltpu.VMEM((S, D), BF16),
            pltpu.VMEM((KD_ROWS, DP), F32),
            pltpu.VMEM((NB, 2 * CB, DP), F32),
            pltpu.VMEM((NB, 2 * CB, D), F32),
            pltpu.VMEM((NB, 2 * CB, D), F32),
            pltpu.VMEM((6, N, D), F32),
            pltpu.VMEM((22, N, DP), F32),
        ],
        compiler_params=pltpu.CompilerParams(vmem_limit_bytes=100 * 1024 * 1024),
    )(xt, wt, wo, ut, B_A_re, B_A_im, B_B_re, B_B_im, B_C_re, B_C_im,
      B_log_dt.reshape(1, D), B_Dskip.reshape(1, D), *consts)
    return out.reshape(1, S, 2 * D)
```

```python
import functools

import jax
import jax.numpy as jnp
import numpy as np
import jax.experimental.pallas as pl
import jax.experimental.pallas.tpu as pltpu

F32 = jnp.float32
BF16 = jnp.bfloat16

S = 2048
D = 448
H = 16
DH = 28
DHP = 32
NG = 4
N = 256
CB = 128
NB = S // CB
KD_ROWS = 656
TQ = 512
NQB = S // TQ
NSTEP = NQB * H
NPS = N // NSTEP
TPC = 128
LOG2E = 1.4426950408889634
DP = 512


def _bf16_round(x):
    x = np.ascontiguousarray(x, dtype=np.float32)
    u = x.view(np.uint32)
    r = (u + 0x7FFF + ((u >> 16) & 1)) & 0xFFFF0000
    return r.astype(np.uint32).view(np.float32)


def _split_hi_lo(m):
    hi = _bf16_round(m)
    lo = _bf16_round(m.astype(np.float64) - hi.astype(np.float64))
    return hi, lo


@functools.lru_cache(maxsize=1)
def _constants():
    th = np.pi * (2 * np.arange(CB) + 1) / (2 * CB)
    t = np.arange(2 * CB)
    ffwd = np.concatenate([np.cos(th[:, None] * t[None, :CB]),
                           -np.sin(th[:, None] * t[None, :CB])], 0)
    finv = np.concatenate([np.cos(th[None, :] * t[CB:, None]),
                           -np.sin(th[None, :] * t[CB:, None])], 1) / CB
    r = _bf16_round(np.arange(S, dtype=np.float32)).astype(np.int64)
    pts = np.concatenate([np.arange(256), 256 + 2 * np.arange(128), 512 + 4 * np.arange(128),
                          1024 + 8 * np.arange(128), [2048]]).astype(np.int64)
    row = np.searchsorted(pts, r)
    assert np.all(pts[row] == r)
    blocks, meta, off = [], [], 0
    for c in range(NB):
        ls = np.arange(CB * (c - 1), CB * (c + 1))
        ls = ls[ls >= 0]
        rows = row[ls]
        b = int(rows.min() // 16) * 16
        n = -(-(int(rows.max()) + 1 - b) // 16) * 16
        g = np.zeros((2 * CB, n), np.float64)
        tt = ls - CB * (c - 1)
        for l_t, rr in zip(tt, rows):
            g[:CB, rr - b] += np.cos(th * l_t)
            g[CB:, rr - b] += -np.sin(th * l_t)
        gh, gl = _split_hi_lo(g)
        w = -(-2 * n // 128) * 128
        blk = np.zeros((2 * CB, w), np.float32)
        blk[:, :n] = gh
        blk[:, n:2 * n] = gl
        blocks.append(blk)
        meta.append((b, n, off))
        off += w
    fh, fl = _split_hi_lo(ffwd)
    ih, il = _split_hi_lo(finv)
    f2 = np.concatenate([fh, fl], 1)
    i3 = np.concatenate([ih, ih, il], 1)
    return (f2, i3, np.concatenate(blocks, 1), tuple(meta))


def _kernel(x_hbm, wt_hbm, wo_hbm, u_hbm, ar_ref, ai_ref, br_ref, bi_ref, cr_ref, ci_ref,
            ldt_ref, dsk_ref, f2_ref, i3_ref, g_hbm,
            out_hbm,
            x_ref, wt_ref, wo_ref, ut_ref, u_ref, g_ref, obuf, in_sems, out_sems,
            q_scr, k_scr, vt_scr, st_scr, ot_scr, oa_scr, kd_scr, uh_scr, kh_scr, yh_scr,
            p_scr, z_scr, *, gmeta):
    copies = [pltpu.make_async_copy(src, dst, in_sems.at[i]) for i, (src, dst) in enumerate(
        ((x_hbm, x_ref), (wt_hbm, wt_ref), (wo_hbm, wo_ref), (u_hbm, ut_ref), (g_hbm, g_ref)))]
    for cp in copies:
        cp.start()

    def pin(tok, x):
        return jnp.where(tok > jnp.inf, tok, x)

    for j, r in enumerate((ar_ref, ai_ref, br_ref, bi_ref, cr_ref, ci_ref)):
        p_scr[j] = r[...].astype(F32).T
    dt = jnp.exp(ldt_ref[...].astype(F32)).astype(BF16).astype(F32)
    srow = jax.lax.broadcasted_iota(jnp.int32, (8, D), 0)
    row128 = jax.lax.broadcasted_iota(jnp.int32, (128, 1), 0)
    z_scr[:, :, pl.ds(384, 128)] = jnp.zeros((22, N, 128), F32)
    kd_scr[...] = jnp.zeros(kd_scr.shape, F32)

    def prep_block(i, tok):
        rows = pl.ds(pl.multiple_of(i * 8, 8), 8)
        dtp = jnp.concatenate([pin(tok, jnp.broadcast_to(dt[:, :128], (8, 128))),
                               jnp.broadcast_to(dt[:, 128:], (8, D - 128))], axis=1)
        zr = dtp * p_scr[0, rows, :]
        zi = dtp * p_scr[1, rows, :]
        dbr = dtp * p_scr[2, rows, :]
        dbi = dtp * p_scr[3, rows, :]
        cr = p_scr[4, rows, :]
        ci = p_scr[5, rows, :]
        z_scr[20, rows, pl.ds(0, D)] = cr * dbr - ci * dbi
        z_scr[21, rows, pl.ds(0, D)] = cr * dbi + ci * dbr

        def ev(m):
            e = jnp.exp(zr * m)
            return e * jnp.cos(zi * m), e * jnp.sin(zi * m)

        def sq(p):
            return p[0] * p[0] - p[1] * p[1], 2.0 * p[0] * p[1]

        p1 = ev(1.0); p2 = sq(p1); p4 = sq(p2)
        p8 = sq(p4); p16 = sq(p8); p32 = sq(p16); p64 = sq(p32)
        p256 = ev(256.0); p512 = sq(p256); p1024 = sq(p512)
        for j, p in enumerate((p1, p2, p4, p8, p16, p32, p64, p256, p512, p1024)):
            z_scr[2 * j, rows, pl.ds(0, D)] = p[0]
            z_scr[2 * j + 1, rows, pl.ds(0, D)] = p[1]

    copies[0].wait(); copies[1].wait(); copies[3].wait()
    u_ref[:, pl.ds(384, 128)] = jnp.zeros((S, 128), BF16)
    PPB = N // 8 // NQB

    def qkv_body(i, c):
        r0 = pl.multiple_of(i * TQ, TQ)
        acc = jnp.dot(wt_ref[...], x_ref[:, pl.ds(r0, TQ)], preferred_element_type=F32)
        for g in range(NG):
            q_scr[g, :, pl.ds(r0, TQ)] = (acc[g * 128:(g + 1) * 128, :]
                                          * (DH ** -0.5 * LOG2E)).astype(BF16)
            k_scr[g, pl.ds(r0, TQ), :] = acc[512 + g * 128:512 + (g + 1) * 128, :].T.astype(BF16)
        vt = acc[1024:, :]
        rowi = jax.lax.broadcasted_iota(jnp.int32, vt.shape, 0)
        vtb = jnp.where((rowi % DHP) == DH, 1.0, vt).astype(BF16)
        for h in range(H):
            vt_scr[h, :, pl.ds(r0, TQ)] = vtb[h * DHP:(h + 1) * DHP, :]
        for j in range(TQ // CB):
            c0 = pl.multiple_of(r0 + j * CB, CB)
            u_ref[pl.ds(c0, CB), pl.ds(0, D)] = ut_ref[:, pl.ds(c0, CB)].astype(F32).T.astype(BF16)
        for j in range(PPB):
            rr = j * (1536 // PPB)
            prep_block(i * PPB + j, acc[rr:rr + 8, 0:128])
        return c

    jax.lax.fori_loop(0, NQB, qkv_body, 0)

    srow128 = jax.lax.broadcasted_iota(jnp.int32, (8, 128), 0)

    def kgen_setup(n, col, pn):
        def row(j):
            return pn(jnp.broadcast_to(z_scr[j, pl.ds(n, 1), :][:, col * 128:(col + 1) * 128],
                                       (8, 128)))

        def cmul(a, b):
            return a[0] * b[0] - a[1] * b[1], a[0] * b[1] + a[1] * b[0]

        def pick(bit, j):
            m = (srow128 & bit) != 0
            return jnp.where(m, row(2 * j), 1.0), jnp.where(m, row(2 * j + 1), 0.0)

        e = cmul(cmul(pick(1, 0), pick(2, 1)), pick(4, 2))
        w = (row(20), row(21))
        segs = []
        for seg in range(4):
            if seg == 0:
                st = w
            else:
                st = cmul(w, (row(2 * (6 + seg)), row(2 * (6 + seg) + 1)))
                e = (e[0] * e[0] - e[1] * e[1], 2.0 * e[0] * e[1])
            x0 = cmul(st, e)
            qr, qi = row(2 * (3 + seg)), row(2 * (3 + seg) + 1)
            x1r = x0[0] * qr - x0[1] * qi
            segs.append((x0[0], x1r, 2.0 * qr, qr * qr + qi * qi))
        return segs

    def kgen_pieces(n0, npiece):
        work = []
        tokens = [None]

        def pn(x):
            return x if tokens[0] is None else pin(tokens[0], x)

        for col in range(DP // 128):
            lanes = pl.ds(col * 128, 128)
            state = {}

            def setup(col=col, state=state):
                state['st'] = [kgen_setup(n0 + j, col, pn) for j in range(NPS)]
                tokens[0] = None

            work.append(setup)
            row = 0
            for seg in range(4):
                nblk = 32 if seg == 0 else (16 if seg < 3 else 17)
                for k in range(nblk):
                    def blk(seg=seg, k=k, nblk=nblk, row=row, lanes=lanes, state=state):
                        st = state['st']
                        if k == 0:
                            state['xs'] = [(s_[seg][0], s_[seg][1]) for s_ in st]
                        xs = [(xp, pn(xc)) for xp, xc in state['xs']]
                        tokens[0] = None
                        tot = xs[0][0]
                        for j in range(1, NPS):
                            tot = tot + xs[j][0]
                        kd_scr[pl.ds(row, 8), lanes] += tot
                        if k + 1 < nblk:
                            state['xs'] = [(xc, st[j][seg][2] * xc - st[j][seg][3] * xp)
                                           if k + 2 < nblk else (xc, xc)
                                           for j, (xp, xc) in enumerate(xs)]
                    work.append(blk)
                    row += 8
        per = -(-len(work) // npiece)
        for p in range(npiece):
            tok = yield
            tokens[0] = tok
            for w in work[p * per:(p + 1) * per]:
                w()
        yield

    def scores(step):
        qb = step // H
        h = step % H
        r0 = pl.multiple_of(qb * TQ, TQ)
        qg = q_scr[h // 4, :, pl.ds(r0, TQ)]
        qm = jnp.where((row128 // DHP) == (h % 4), qg, jnp.zeros_like(qg))
        st = jnp.dot(k_scr[h // 4], qm, preferred_element_type=F32)
        st_scr[step % 2] = st
        return jnp.max(st, axis=0, keepdims=True)

    def step_body(step, mx):
        qb = step // H
        h = step % H
        r0 = pl.multiple_of(qb * TQ, TQ)
        nstep = jnp.minimum(step + 1, NSTEP - 1)
        pieces = kgen_pieces(step * NPS, TPC)
        next(pieces)
        ulanes = pl.ds(pl.multiple_of((step % 4) * 128, 128), 128)
        ub = u_ref[pl.ds(pl.multiple_of((step // 4) * CB, CB), CB), ulanes]
        uh_scr[step // 4, :, ulanes] = jnp.dot(f2_ref[...], jnp.concatenate([ub, ub], axis=0),
                                               preferred_element_type=F32)
        pt = jnp.exp2(st_scr[step % 2] - mx).astype(BF16)
        ot = jnp.dot(vt_scr[h], pt, preferred_element_type=F32)
        mx_next = scores(nstep)
        for tk in range(TPC):
            pieces.send(st_scr[nstep % 2, pl.ds(tk * (S // TPC), 8), pl.ds(0, 128)])
        ot = ot * (1.0 / ot[DH:DH + 1, :])
        ot_scr[pl.ds(pl.multiple_of(h * DHP, DHP), DHP), :] = ot.astype(BF16)

        @pl.when(h == H - 1)
        def _():
            oa = jax.lax.dot_general(ot_scr[...], wo_ref[...], (((0,), (0,)), ((), ())),
                                     preferred_element_type=F32)
            oa_scr[pl.ds(r0, TQ), :] = oa.astype(BF16)
        return mx_next

    copies[2].wait()
    jax.lax.fori_loop(0, NSTEP, step_body, scores(0))

    tail = kd_scr[pl.ds(640, 8), pl.ds(0, D)]
    kd_scr[pl.ds(640, 8), pl.ds(0, D)] = jnp.where(srow == 0, tail, 0.0)

    copies[4].wait()

    for c in range(NB):
        b, n, off = gmeta[c]
        kd = kd_scr[pl.ds(b, n), pl.ds(0, D)]
        kd_hi = kd.astype(BF16)
        kd_lo = (kd - kd_hi.astype(F32)).astype(BF16)
        g2 = g_ref[:, pl.ds(off, 2 * n)]
        kh_scr[c] = (jnp.dot(g2, jnp.concatenate([kd_hi, kd_hi], axis=0),
                             preferred_element_type=F32)
                     + jnp.dot(g2[:, :n], kd_lo, preferred_element_type=F32))

    dsk = dsk_ref[...].astype(F32)

    def acc_body(rb, c):
        rows_r = pl.ds(pl.multiple_of(rb * 8, 8), 8)
        rows_i = pl.ds(pl.multiple_of(CB + rb * 8, 8), 8)
        for i in range(NB):
            yr = yi = None
            for cc in range(i + 1):
                kr = kh_scr[cc, rows_r, :]
                ki = kh_scr[cc, rows_i, :]
                ur = uh_scr[i - cc, rows_r, pl.ds(0, D)]
                ui = uh_scr[i - cc, rows_i, pl.ds(0, D)]
                tr_ = kr * ur - ki * ui
                ti_ = kr * ui + ki * ur
                yr = tr_ if yr is None else yr + tr_
                yi = ti_ if yi is None else yi + ti_
            yh_scr[i, rows_r, :] = yr
            yh_scr[i, rows_i, :] = yi
        return c

    jax.lax.fori_loop(0, CB // 8, acc_body, 0)

    def out_copy(i, slot):
        return pltpu.make_async_copy(obuf.at[slot],
                                     out_hbm.at[pl.ds(pl.multiple_of(i * CB, CB), CB), :],
                                     out_sems.at[slot])

    def conv_body(i, c):
        slot = i % 2
        yh = yh_scr[i]
        yh_hi = yh.astype(BF16)
        yh_lo = (yh - yh_hi.astype(F32)).astype(BF16)
        y = jnp.dot(i3_ref[...], jnp.concatenate([yh_hi, yh_lo, yh_hi], axis=0),
                    preferred_element_type=F32)
        r0 = pl.multiple_of(i * CB, CB)
        ub = u_ref[pl.ds(r0, CB), pl.ds(0, D)].astype(F32)
        t1 = (ub * dsk).astype(BF16).astype(F32)
        ob = (y.astype(BF16).astype(F32) + t1).astype(BF16)

        @pl.when(i >= 2)
        def _():
            out_copy(i - 2, slot).wait()

        obuf[slot] = jnp.concatenate([oa_scr[pl.ds(r0, CB), :], ob], axis=1)
        out_copy(i, slot).start()
        return c

    jax.lax.fori_loop(0, NB, conv_body, 0)
    out_copy(NB - 2, 0).wait()
    out_copy(NB - 1, 1).wait()


@jax.jit
def pallas_concat_heads__mha_block__ssm_conv_s4__prompt_kernel(
    A_x, A_wqkv, A_wo, B_u, B_A_re, B_A_im, B_B_re, B_B_im, B_C_re, B_C_im, B_log_dt, B_Dskip,
):
    f2, i3, gt, gmeta = _constants()
    xt = A_x.reshape(S, D).T
    ut = B_u.reshape(S, D).T
    wt = jnp.pad(A_wqkv.T.reshape(3 * H, DH, D), ((0, 0), (0, DHP - DH), (0, 0))).reshape(3 * H * DHP, D)
    wo = jnp.pad(A_wo.reshape(H, DH, D), ((0, 0), (0, DHP - DH), (0, 0))).reshape(H * DHP, D)
    consts = [jnp.asarray(c, dtype=BF16) for c in (f2, i3, gt)]
    hbm = pl.BlockSpec(memory_space=pl.ANY)
    vmem = pl.BlockSpec(memory_space=pltpu.VMEM)
    out = pl.pallas_call(
        functools.partial(_kernel, gmeta=gmeta),
        out_shape=jax.ShapeDtypeStruct((S, 2 * D), BF16),
        in_specs=[hbm] * 4 + [vmem] * 10 + [hbm],
        out_specs=hbm,
        scratch_shapes=[
            pltpu.VMEM((D, S), BF16),
            pltpu.VMEM((3 * H * DHP, D), BF16),
            pltpu.VMEM((H * DHP, D), BF16),
            pltpu.VMEM((D, S), BF16),
            pltpu.VMEM((S, DP), BF16),
            pltpu.VMEM(gt.shape, BF16),
            pltpu.VMEM((2, CB, 2 * D), BF16),
            pltpu.SemaphoreType.DMA((5,)),
            pltpu.SemaphoreType.DMA((2,)),
            pltpu.VMEM((NG, 128, S), BF16),
            pltpu.VMEM((NG, S, 128), BF16),
            pltpu.VMEM((H, DHP, S), BF16),
            pltpu.VMEM((2, S, TQ), F32),
            pltpu.VMEM((H * DHP, TQ), BF16),
            pltpu.VMEM((S, D), BF16),
            pltpu.VMEM((KD_ROWS, DP), F32),
            pltpu.VMEM((NB, 2 * CB, DP), F32),
            pltpu.VMEM((NB, 2 * CB, D), F32),
            pltpu.VMEM((NB, 2 * CB, D), F32),
            pltpu.VMEM((6, N, D), F32),
            pltpu.VMEM((22, N, DP), F32),
        ],
        compiler_params=pltpu.CompilerParams(vmem_limit_bytes=100 * 1024 * 1024),
    )(xt, wt, wo, ut, B_A_re, B_A_im, B_B_re, B_B_im, B_C_re, B_C_im,
      B_log_dt.reshape(1, D), B_Dskip.reshape(1, D), *consts)
    return out.reshape(1, S, 2 * D)
```
